```python
import os as _os
_os.environ.setdefault("JAX_PLATFORMS", "cpu")
import jax
import jax.numpy as jnp

def _softmax(x, axis=-1):
    return jax.nn.softmax(x, axis=axis)
def _gelu(x):
    return jax.nn.gelu(x, approximate=True)
def _silu(x):
    return jax.nn.silu(x)
def _sigmoid(x):
    return jax.nn.sigmoid(x)
def _layernorm(x, axis=-1, eps=1e-5):
    m = jnp.mean(x, axis=axis, keepdims=True)
    v = jnp.var(x, axis=axis, keepdims=True)
    return (x - m) / jnp.sqrt(v + eps)
def _scatter_add(tgt, idx, src, axis=0):
    return tgt.at[idx].add(src)
def _segment_sum(src, seg, n):
    return jax.ops.segment_sum(src, seg, n)
class _Rng:
    def __init__(self, key):
        self._k = key
    def _next(self):
        self._k, sub = jax.random.split(self._k)
        return sub
    def normal(self, shape):
        return jax.random.normal(self._next(), shape, dtype=jnp.bfloat16)
    def randint(self, lo, hi, shape):
        return jax.random.randint(self._next(), shape, lo, hi, dtype=jnp.int32)
    def uniform(self, shape, lo=0.0, hi=1.0):
        return jax.random.uniform(self._next(), shape, jnp.bfloat16, lo, hi)
    def permutation(self, n):
        return jax.random.permutation(self._next(), n)


kernel_name = 'concat_heads__gqa_block_cached__gqa_block_cached__near_ridge'

def setup_inputs():
    _rng = _Rng(jax.random.key(int.from_bytes(__import__("os").urandom(4), "little")))
    _w = (lambda a: (lambda t: t.astype(jnp.bfloat16) if jnp.issubdtype(t.dtype, jnp.floating) else t)(jnp.asarray(a)))
    def _A_setup():
        B, Sq, D = 8, 128, 576
        Hq, Hkv, Sk, Dh = 32, 16, 512, 128
        assert Hq % Hkv == 0, (Hq, Hkv)
        return {
            "x": _w((lambda *s: _rng.normal(s) * 0.8)(B, Sq, D)),
            "k_cache": _w((lambda *s: _rng.normal(s) * 0.8)(B, Hkv, Sk, Dh)),
            "v_cache": _w((lambda *s: _rng.normal(s) * 0.05)(B, Hkv, Sk, Dh)),
            "wq": _w((lambda *s: _rng.normal(s) * 0.8)(D, Hq * Dh) * (D ** -0.5)),
            "wo": _w((lambda *s: _rng.normal(s) * 0.05)(Hq * Dh, D) * ((Hq * Dh) ** -0.5)),
        }
    _A_in = _A_setup()

    def _B_setup():
        B, Sq, D = 8, 128, 576
        Hq, Hkv, Sk, Dh = 32, 16, 512, 128
        assert Hq % Hkv == 0, (Hq, Hkv)
        return {
            "x": _w((lambda *s: _rng.normal(s) * 0.8)(B, Sq, D)),
            "k_cache": _w((lambda *s: _rng.normal(s) * 0.8)(B, Hkv, Sk, Dh)),
            "v_cache": _w((lambda *s: _rng.normal(s) * 0.05)(B, Hkv, Sk, Dh)),
            "wq": _w((lambda *s: _rng.normal(s) * 0.8)(D, Hq * Dh) * (D ** -0.5)),
            "wo": _w((lambda *s: _rng.normal(s) * 0.05)(Hq * Dh, D) * ((Hq * Dh) ** -0.5)),
        }
    _B_in = _B_setup()

    return {
        "A_x": _A_in["x"],
        "A_k_cache": _A_in["k_cache"],
        "A_v_cache": _A_in["v_cache"],
        "A_wq": _A_in["wq"],
        "A_wo": _A_in["wo"],
        "B_x": _B_in["x"],
        "B_k_cache": _B_in["k_cache"],
        "B_v_cache": _B_in["v_cache"],
        "B_wq": _B_in["wq"],
        "B_wo": _B_in["wo"],
    }

def reference(A_x, A_k_cache, A_v_cache, A_wq, A_wo, B_x, B_k_cache, B_v_cache, B_wq, B_wo):
    def _A_ref(x, k_cache, v_cache, wq, wo):
        B, Sq, D = x.shape
        Hq, Dh = 32, 128
        Hkv = k_cache.shape[1]
        rep = Hq // Hkv
        q = (lambda x, *d: x.transpose(*d))((x @ wq).reshape(B, Sq, Hq, Dh), 0, 2, 1, 3)
        k = jnp.repeat(k_cache, rep, axis=1)
        v = jnp.repeat(v_cache, rep, axis=1)
        scores = jnp.einsum("bhqd,bhkd->bhqk", q, k) * (Dh ** -0.5)
        p = _softmax(scores, axis=-1)
        o = jnp.einsum("bhqk,bhkd->bhqd", p, v)
        return (lambda x, *d: x.transpose(*d))(o, 0, 2, 1, 3).reshape(B, Sq, Hq * Dh) @ wo

    def _B_ref(x, k_cache, v_cache, wq, wo):
        B, Sq, D = x.shape
        Hq, Dh = 32, 128
        Hkv = k_cache.shape[1]
        rep = Hq // Hkv
        q = (lambda x, *d: x.transpose(*d))((x @ wq).reshape(B, Sq, Hq, Dh), 0, 2, 1, 3)
        k = jnp.repeat(k_cache, rep, axis=1)
        v = jnp.repeat(v_cache, rep, axis=1)
        scores = jnp.einsum("bhqd,bhkd->bhqk", q, k) * (Dh ** -0.5)
        p = _softmax(scores, axis=-1)
        o = jnp.einsum("bhqk,bhkd->bhqd", p, v)
        return (lambda x, *d: x.transpose(*d))(o, 0, 2, 1, 3).reshape(B, Sq, Hq * Dh) @ wo

    a = _A_ref(A_x, A_k_cache, A_v_cache, A_wq, A_wo)
    b = _B_ref(B_x, B_k_cache, B_v_cache, B_wq, B_wo)
    return jnp.concatenate([a, b], axis=-1)
```

```python
import functools, math
import jax, jax.numpy as jnp, numpy as np
import jax.experimental.pallas as pl
import jax.experimental.pallas.tpu as pltpu

B, SQ, D, HQ, HKV, SK, DH = 8, 128, 576, 32, 16, 512, 128
DP = 640
NT = lambda a, b: jax.lax.dot_general(a, b, (((1,), (1,)), ((), ())), preferred_element_type=jnp.float32)
NN = lambda a, b: jnp.dot(a, b, preferred_element_type=jnp.float32)

def make(BB=8, outT=True, qall=False, recip_approx=False):
    NBG = B // BB
    C = float(DH ** -0.5 * math.log2(math.e))

    def kernel(xa_ref, ka_ref, va_ref, wqa_ref, woa_ref, xb_ref, kb_ref, vb_ref, wqb_ref, wob_ref,
               o_ref, xs_ref, acc_ref):
        g = pl.program_id(0)
        bg = pl.program_id(1)
        xrefs = (xa_ref, xb_ref)

        @pl.when((g == 0) & (bg == 0))
        def _():
            for br in range(2):
                for b in range(B):
                    for j in range(5):
                        if j < 4:
                            blk = xrefs[br][b, j * 128:(j + 1) * 128, :]
                        else:
                            blk = jnp.concatenate([xrefs[br][b, 512:576, :], jnp.zeros((64, 128), jnp.bfloat16)], axis=0)
                        xs_ref[br, b * 128:(b + 1) * 128, j * 128:(j + 1) * 128] = blk.T
            acc_ref[...] = jnp.zeros(acc_ref.shape, acc_ref.dtype)

        for br, (k_ref, v_ref, wq_ref, wo_ref) in enumerate(((ka_ref, va_ref, wqa_ref, woa_ref), (kb_ref, vb_ref, wqb_ref, wob_ref))):
            wq = jnp.concatenate([wq_ref[...], jnp.zeros((64, 256), jnp.bfloat16)], axis=0)
            for bi in range(BB):
                b = bg * BB + bi
                row0 = pl.multiple_of(b * 128, 128)
                x = xs_ref[br, pl.ds(row0, 128), :]
                q = (NN(x, wq) * C).astype(jnp.bfloat16)
                q2 = jnp.concatenate([q[:, :128], q[:, 128:]], axis=0)
                s = NT(q2, k_ref[bi, 0])
                m = jnp.max(s, axis=-1, keepdims=True)
                p = jnp.exp2(s - m)
                l = jnp.sum(p, axis=-1, keepdims=True)
                o = NN(p.astype(jnp.bfloat16), v_ref[bi, 0])
                o = (o * pl.reciprocal(l, approx=recip_approx)).astype(jnp.bfloat16)
                if outT:
                    r = NT(wo_ref[:, 0:128], o[0:128]) + NT(wo_ref[:, 128:256], o[128:256])
                    acc_ref[br, b] += r
                else:
                    o2 = jnp.concatenate([o[0:128], o[128:256]], axis=1)
                    r = NT(o2, wo_ref[...])
                    acc_ref[br, b] += r

        @pl.when((g == HKV - 1))
        def _():
            for bi in range(BB):
                b = bg * BB + bi
                if outT:
                    parts = []
                    full = jnp.concatenate([acc_ref[0, b], acc_ref[1, b]], axis=0)
                    for j in range(9):
                        o_ref[bi, :, j * 128:(j + 1) * 128] = full[j * 128:(j + 1) * 128, :].T.astype(jnp.bfloat16)
                else:
                    full = jnp.concatenate([acc_ref[0, b], acc_ref[1, b]], axis=1)
                    o_ref[bi] = full.astype(jnp.bfloat16)

    x_spec = pl.BlockSpec((B, D, SQ), lambda g, bg: (0, 0, 0))
    kv_spec = pl.BlockSpec((BB, 1, SK, DH), lambda g, bg: (bg, g, 0, 0))
    w_spec = pl.BlockSpec((D, 256), lambda g, bg: (0, g))
    out_spec = pl.BlockSpec((BB, SQ, 2 * D), lambda g, bg: (jnp.where(g == HKV - 1, bg, 0), 0, 0))
    acc_shape = (2, B, D, SQ) if outT else (2, B, SQ, D)

    @jax.jit
    def f(A_x, A_k, A_v, A_wq, A_wo, B_x, B_k, B_v, B_wq, B_wo):
        return pl.pallas_call(
            kernel,
            grid=(HKV, NBG),
            in_specs=[x_spec, kv_spec, kv_spec, w_spec, w_spec] * 2,
            out_specs=out_spec,
            out_shape=jax.ShapeDtypeStruct((B, SQ, 2 * D), jnp.bfloat16),
            scratch_shapes=[pltpu.VMEM((2, B * SQ, DP), jnp.bfloat16), pltpu.VMEM(acc_shape, jnp.float32)],
            compiler_params=pltpu.CompilerParams(dimension_semantics=("arbitrary", "arbitrary"),
                                                 vmem_limit_bytes=100 * 1024 * 1024),
        )(A_x.transpose(0, 2, 1), A_k, A_v, A_wq, A_wo.T, B_x.transpose(0, 2, 1), B_k, B_v, B_wq, B_wo.T)
    return f


_impl = make(BB=8, outT=False)


@jax.jit
def pallas_concat_heads__gqa_block_cached__gqa_block_cached__near_ridge_kernel(
    A_x: jax.Array,
    A_k_cache: jax.Array,
    A_v_cache: jax.Array,
    A_wq: jax.Array,
    A_wo: jax.Array,
    B_x: jax.Array,
    B_k_cache: jax.Array,
    B_v_cache: jax.Array,
    B_wq: jax.Array,
    B_wo: jax.Array,
):
    return _impl(A_x, A_k_cache, A_v_cache, A_wq, A_wo, B_x, B_k_cache, B_v_cache, B_wq, B_wo)
```

```python
import functools, math
import jax, jax.numpy as jnp, numpy as np
import jax.experimental.pallas as pl
import jax.experimental.pallas.tpu as pltpu
B, SQ, D, HQ, HKV, SK, DH = 8, 128, 576, 32, 16, 512, 128
DP = 640
U = 16
NL = 3
def NT(a, b): return jax.lax.dot_general(a, b, (((1,), (1,)), ((), ())), preferred_element_type=jnp.float32)
def NN(a, b): return jnp.dot(a, b, preferred_element_type=jnp.float32)

def interleave(units, xfill, yfill, pend):
    seq = []; pend = list(pend); xfill = list(xfill); yfill = list(yfill)
    units = list(units); n = len(units)
    for i, u in enumerate(units):
        seq.append(("S", u))
        if len(pend) >= 2: seq.append(("O", pend.pop(0)))
        elif xfill: seq.append(xfill.pop(0))
        seq.append(("V", u)); pend.append(u)
        while yfill and len(yfill) >= n - i: seq.append(yfill.pop(0))
    assert not xfill and not yfill, (xfill, yfill)
    return seq, pend

def make(recip="newton", osplit=2, NG=16, scopes=False, pin=0, flag=2, startpos=2, q0lag=0, flags=None):
    C = float(DH ** -0.5 * math.log2(math.e))
    bf = jnp.bfloat16
    NPOOL = 64 + 18

    def kernel(xa, ka, va, wqa, woa, xb, kb, vb, wqb, wob, out_hbm,
               xT, xs, qs, pool, wv, acc, sem_g, sem_kv, sem_w, sem_o):
        x_h = (xa, xb); k_h = (ka, kb); v_h = (va, vb); wq_h = (wqa, wqb); wo_h = (woa, wob)
        def col(g):
            c = g * 256
            return pl.ds(c if isinstance(c, int) else pl.multiple_of(c, 256), 256)
        def cp_kv(g, slot, which, br, b0, b1, sem):
            src = (k_h, v_h)[which][br]
            return pltpu.make_async_copy(src.at[pl.ds(b0, b1 - b0), g], pool.at[pl.ds(slot * 32 + which * 16 + br * B + b0, b1 - b0)], sem)
        def cp_w(g, slot, which, br, sem):
            src = (wq_h, wo_h)[which][br]
            return pltpu.make_async_copy(src.at[:, col(g)], wv.at[slot, which, br], sem)
        def cp_x(br, b0, b1, sem):
            return pltpu.make_async_copy(x_h[br].at[pl.ds(b0, b1 - b0)], xT.at[pl.ds(br * B + b0, b1 - b0)], sem)
        def tile_loc(b, j):
            t = b * 9 + j
            return 64 + t // 4, (t % 4) * 128
        def cp_out(b, j):
            r, s = tile_loc(b, j)
            return pltpu.make_async_copy(pool.at[r, pl.ds(s, 128), :], out_hbm.at[b, :, pl.ds(j * 128, 128)], sem_o.at[0])
        def next_copies(g, slot):
            c = []
            gq = g + 1
            gq = min(gq, HKV - 1) if isinstance(gq, int) else jnp.minimum(gq, HKV - 1)
            for br in range(2):
                for which in range(2):
                    c.append(cp_kv(g, slot, which, br, 0, B, sem_kv.at[slot]))
                c.append(cp_w(g, slot, 1, br, sem_w.at[slot]))
                c.append(cp_w(gq, slot, 0, br, sem_w.at[slot]))
            return c
        def wait_block(slot):
            pltpu.make_async_copy(pool.at[pl.ds(slot * 32, 32)], pool.at[pl.ds(slot * 32, 32)], sem_kv.at[slot]).wait()
            pltpu.make_async_copy(wv.at[slot], wv.at[slot], sem_w.at[slot]).wait()
        def recip_fn(l):
            if recip == "exact": return pl.reciprocal(l, approx=False)
            r = pl.reciprocal(l, approx=True)
            if recip == "newton": r = r * (2.0 - l * r)
            return r
        def scoped(name, fn):
            if scopes:
                with jax.named_scope(name): fn()
            else: fn()

        def block(slot, first, last, hooks, kvslot=None):
            st = [dict() for _ in range(U)]
            kvs = slot if kvslot is None else kvslot
            def hook(name):
                for t in hooks.get(name, ()): t()
            def qproj(x, wslot, br, u):
                wq = jnp.concatenate([wv[wslot, 0, br], jnp.zeros((64, 256), bf)], axis=0)
                q = (NN(x, wq) * C).astype(bf)
                qs[u, 0:128, :] = q[:, :128]
                qs[u, 128:256, :] = q[:, 128:]
            def TQ(u):
                tiles = []
                for j in range(5):
                    if j < 4: blk = xT[u, j * 128:(j + 1) * 128, :]
                    else: blk = jnp.concatenate([xT[u, 512:576, :], jnp.zeros((64, 128), bf)], axis=0)
                    tiles.append(blk.T)
                x = jnp.concatenate(tiles, axis=1)
                xs[u] = x
                qproj(x, 1, u // B, u)
            def Qn(u): qproj(xs[u], slot, u // B, u)
            def Qc(u): qproj(xs[u], 1 - slot, u // B, u)
            def S(u):
                s = NT(qs[u], pool[kvs * 32 + u])
                m = jnp.max(s, axis=-1, keepdims=True)
                p = jnp.exp2(s - m)
                st[u]["l"] = jnp.sum(p, axis=-1, keepdims=True)
                st[u]["p"] = p.astype(bf)
                hook(("S", u))
            def V(u):
                o = NN(st[u].pop("p"), pool[kvs * 32 + 16 + u])
                st[u]["o"] = (o * recip_fn(st[u].pop("l"))).astype(bf)
            def O(u):
                br, b = u // B, u % B
                o = st[u].pop("o")
                RR = D // osplit
                parts = []
                for r in range(osplit):
                    rows = slice(r * RR, (r + 1) * RR)
                    res = NT(wv[slot, 1, br, rows, 0:128], o[0:128]) + NT(wv[slot, 1, br, rows, 128:256], o[128:256])
                    if not first: res = acc[u, rows, :] + res
                    if last: parts.append(res)
                    else: acc[u, rows, :] = res
                if last: st[u]["fin"] = jnp.concatenate(parts, axis=0)
            def put(b, j, t):
                r, s = tile_loc(b, j)
                pool[r, s:s + 128, :] = t.T.astype(bf)
                cp_out(b, j).start()
            def F(u):
                br, b = u // B, u % B
                fin = st[u].pop("fin")
                if br == 0:
                    acc[u, 512:576, :] = fin[512:576]
                    for j in range(4): put(b, j, fin[j * 128:(j + 1) * 128, :])
                else:
                    put(b, 4, jnp.concatenate([acc[b, 512:576, :], fin[0:64]], axis=0))
                    for j in range(4): put(b, 5 + j, fin[64 + j * 128:64 + (j + 1) * 128, :])
            fns = {"Qn": Qn, "Qc": Qc, "S": S, "V": V, "O": O, "TQ": TQ, "F": F}
            def emit(seq):
                for k, u in seq: fns[k](u)
            if first:
                hook(0); emit([("TQ", u) for u in range(0, 4)])
                hook(1); emit([("TQ", u) for u in range(4, 8)])
                hook(2)
                s1, pend = interleave(range(0, 8), [("Qn", 0), ("Qn", 1)], [("Qn", u) for u in range(2, 8 - q0lag)], [])
                cut = s1.index(("S", 4))
                emit(s1[:cut]); hook(3); emit(s1[cut:])
                hook(4); emit([("TQ", u) for u in range(8, 16)])
                hook(5)
                s2, pend = interleave(range(8, 16), [], [("Qn", u) for u in range(8 - q0lag, U - NL)], pend)
                emit(s2); emit([("O", u) for u in pend])
                return
            hook("top")
            qc = [("Qc", u) for u in range(U - NL, U)]
            if not last:
                s1, pend = interleave(range(U), qc[1:], [("Qn", u) for u in range(U - NL)], [])
                s1 = qc[:1] + s1 + [("O", u) for u in pend]
            else:
                s1 = [qc[0], ("S", 0), qc[1], ("S", 1), qc[2], ("V", 0)]
                for u in range(1, U):
                    if u + 1 < U: s1 += [("S", u + 1), ("O", u - 1)]
                    s1.append(("V", u))
                s1 += [("O", U - 2), ("O", U - 1)]
                out = []; due = []
                for e in s1:
                    out.append(e)
                    due = [(c - 1, u) for c, u in due]
                    while due and due[0][0] <= 0: out.append(("F", due.pop(0)[1]))
                    if e[0] == "O": due.append((flag, e[1]))
                s1 = out + [("F", u) for _, u in due]
            emit(s1)

        sg = lambda i: sem_g.at[i]
        G = [
            [cp_w(0, 1, 0, 0, sg(0))] + [cp_x(0, b, b + 1, sg(0)) for b in range(0, 4)],
            [cp_x(0, 4, 8, sg(1))],
            [cp_w(0, 0, 1, 0, sg(2)), cp_kv(0, 0, 0, 0, 0, 4, sg(2)), cp_kv(0, 0, 1, 0, 0, 4, sg(2)), cp_w(1, 0, 0, 0, sg(2))],
            [cp_kv(0, 0, 0, 0, 4, 8, sg(3)), cp_kv(0, 0, 1, 0, 4, 8, sg(3))],
            [cp_w(0, 1, 0, 1, sg(4)), cp_x(1, 0, 8, sg(4))],
            [cp_w(0, 0, 1, 1, sg(5)), cp_kv(0, 0, 0, 1, 0, 8, sg(5)), cp_kv(0, 0, 1, 1, 0, 8, sg(5)), cp_w(1, 0, 0, 1, sg(5))],
        ]
        nxt1 = next_copies(1, 1)
        def startall(cs):
            for c in cs: c.start()
        def waitall(cs):
            for c in cs: c.wait()
        h = {}
        seq = G + [nxt1[:4], nxt1[4:]]
        for i in range(6):
            h[i] = [functools.partial(scoped, f"wG{i}", functools.partial(waitall, G[i])), functools.partial(startall, seq[i + 2])]
        startall(G[0]); startall(G[1])
        block(0, True, False, h)

        def body(g, slot):
            nx = next_copies(g + 1, 1 - slot)
            hk = {"top": [functools.partial(scoped, "wtop_loop", functools.partial(wait_block, slot))],
                  ("S", startpos - 1): [functools.partial(startall, nx[:4])],
                  ("S", startpos): [functools.partial(startall, nx[4:])]}
            block(slot, False, False, hk)
            return 1 - slot
        dslot = jax.lax.fori_loop(1, NG - 1, body, 1) if NG > 2 else 1
        ls = (NG - 1) % 2
        hk = {"top": [functools.partial(scoped, "wtop_last", functools.partial(wait_block, ls))]}
        block(ls, False, True, hk, kvslot=(dslot if pin else None))
        scoped("wout", lambda: pltpu.make_async_copy(pool.at[pl.ds(64, 18)], pool.at[pl.ds(64, 18)], sem_o.at[0]).wait())

    hbm = pl.BlockSpec(memory_space=pltpu.HBM)
    @jax.jit
    def f(A_x, A_k, A_v, A_wq, A_wo, B_x, B_k, B_v, B_wq, B_wo):
        return pl.pallas_call(kernel, in_specs=[hbm] * 10, out_specs=hbm,
            out_shape=jax.ShapeDtypeStruct((B, SQ, 2 * D), bf),
            scratch_shapes=[pltpu.VMEM((U, D, SQ), bf), pltpu.VMEM((U, SQ, DP), bf), pltpu.VMEM((U, 256, DH), bf),
                            pltpu.VMEM((NPOOL, SK, DH), bf), pltpu.VMEM((2, 2, 2, D, 256), bf),
                            pltpu.VMEM((U, D, SQ), jnp.float32),
                            pltpu.SemaphoreType.DMA((6,)), pltpu.SemaphoreType.DMA((2,)), pltpu.SemaphoreType.DMA((2,)),
                            pltpu.SemaphoreType.DMA((1,))],
            compiler_params=pltpu.CompilerParams(vmem_limit_bytes=100 * 1024 * 1024, flags=flags),
        )(A_x.transpose(0, 2, 1), A_k, A_v, A_wq, A_wo.T, B_x.transpose(0, 2, 1), B_k, B_v, B_wq, B_wo.T)
    return f

_impl = make(pin=1, flag=2)


@jax.jit
def pallas_concat_heads__gqa_block_cached__gqa_block_cached__near_ridge_kernel(
    A_x: jax.Array,
    A_k_cache: jax.Array,
    A_v_cache: jax.Array,
    A_wq: jax.Array,
    A_wo: jax.Array,
    B_x: jax.Array,
    B_k_cache: jax.Array,
    B_v_cache: jax.Array,
    B_wq: jax.Array,
    B_wo: jax.Array,
):
    return _impl(A_x, A_k_cache, A_v_cache, A_wq, A_wo, B_x, B_k_cache, B_v_cache, B_wq, B_wo)
```

```python
import functools
import math

import jax
import jax.numpy as jnp
import jax.experimental.pallas as pl
import jax.experimental.pallas.tpu as pltpu

_B, _SQ, _D, _HKV, _SK, _DH = 8, 128, 576, 16, 512, 128
_DP = 640
_HP = 2 * _DH
_QSCALE = float(_DH ** -0.5 * math.log2(math.e))
_OSPLIT = 4
_NTILE = 2 * _D // 128
_KV_ROWS = 64
_OUT_ROWS = _B * _NTILE // 4
_FIN_LAG = 3
_BF = jnp.bfloat16


def _nt(a, b):
    return jax.lax.dot_general(a, b, (((1,), (1,)), ((), ())), preferred_element_type=jnp.float32)


def _nn(a, b):
    return jnp.dot(a, b, preferred_element_type=jnp.float32)


def _interleave(units, xfill, yfill, pend):
    seq, pend, xfill, yfill, units = [], list(pend), list(xfill), list(yfill), list(units)
    for i, u in enumerate(units):
        seq.append(("S", u))
        if len(pend) >= 2:
            seq.append(("O", pend.pop(0)))
        elif xfill:
            seq.append(xfill.pop(0))
        seq.append(("V", u))
        pend.append(u)
        while yfill and len(yfill) >= len(units) - i:
            seq.append(yfill.pop(0))
    return seq + xfill, pend


def _kernel(xa, ka, va, wqa, woa, xb, kb, vb, wqb, wob, out_hbm,
            x_t, xs, qs, q0, pool, wv, w0, acc, sem_g, sem_kv, sem_w, sem_o):
    x_h, k_h, v_h, wq_h, wo_h = (xa, xb), (ka, kb), (va, vb), (wqa, wqb), (woa, wob)

    def cols(g):
        c = g * _HP
        return pl.ds(c if isinstance(c, int) else pl.multiple_of(c, _HP), _HP)

    def cp_kv(g, slot, which, br, b0, b1, sem):
        src = (k_h, v_h)[which][br].at[pl.ds(b0, b1 - b0), g]
        return pltpu.make_async_copy(src, pool.at[pl.ds(slot * 32 + which * 16 + br * _B + b0, b1 - b0)], sem)

    def cp_w(g, which, br, dst, sem):
        return pltpu.make_async_copy((wq_h, wo_h)[which][br].at[:, cols(g)], dst, sem)

    def cp_x(br, b0, b1, sem):
        return pltpu.make_async_copy(x_h[br].at[pl.ds(b0, b1 - b0)], x_t.at[pl.ds(br * _B + b0, b1 - b0)], sem)

    def tile_loc(b, j):
        t = b * _NTILE + j
        return _KV_ROWS + t // 4, (t % 4) * 128

    def block_copies(j, slot):
        jn = j + 1
        jn = min(jn, _HKV - 1) if isinstance(jn, int) else jnp.minimum(jn, _HKV - 1)
        c = []
        for br, g in ((1, j), (0, jn)):
            c += [cp_kv(g, slot, which, br, 0, _B, sem_kv.at[slot]) for which in range(2)]
            c.append(cp_w(g, 1, br, wv.at[slot, 1, br], sem_w.at[slot]))
            c.append(cp_w(jn, 0, 1 - br, wv.at[slot, 0, 1 - br], sem_w.at[slot]))
        return c

    def wait_block(slot):
        rows = pool.at[pl.ds(slot * 32, 32)]
        pltpu.make_async_copy(rows, rows, sem_kv.at[slot]).wait()
        pltpu.make_async_copy(wv.at[slot], wv.at[slot], sem_w.at[slot]).wait()

    def start_all(cs):
        for c in cs:
            c.start()

    def wait_all(cs):
        for c in cs:
            c.wait()

    units, live, hooks = {}, {}, {}

    def hook(name):
        for t in hooks.pop(name, ()):
            t()

    def qproj(x, wq_ref, q_ref, i):
        wq = jnp.concatenate([wq_ref[...], jnp.zeros((_DP - _D, _HP), _BF)], axis=0)
        q = (_nn(x, wq) * _QSCALE).astype(_BF)
        q_ref[i, 0:_SQ, :] = q[:, :_DH]
        q_ref[i, _SQ:2 * _SQ, :] = q[:, _DH:]

    def stage_tq(a):
        br, b, wq_ref, q_ref, i = a
        u = br * _B + b
        tiles = [x_t[u, j * 128:(j + 1) * 128, :].T for j in range(4)]
        tail = jnp.concatenate([x_t[u, 512:_D, :], jnp.zeros((_DP - _D, _SQ), _BF)], axis=0)
        x = jnp.concatenate(tiles + [tail.T], axis=1)
        xs[u] = x
        qproj(x, wq_ref, q_ref, i)

    def stage_q(a):
        br, b, wq_ref, q_ref, i = a
        qproj(xs[br * _B + b], wq_ref, q_ref, i)

    def stage_s(k):
        d = units[k]
        s = _nt(d["q"][d["qi"]], pool[d["kv"] * 32 + d["u"]])
        p = jnp.exp2(s - jnp.max(s, axis=-1, keepdims=True))
        live[k] = {"l": jnp.sum(p, axis=-1, keepdims=True), "p": p.astype(_BF)}
        hook(("S", k))

    def stage_v(k):
        o = _nn(live[k].pop("p"), pool[units[k]["kv"] * 32 + 16 + units[k]["u"]])
        den = live[k].pop("l")
        r = pl.reciprocal(den, approx=True)
        r = r * (2.0 - den * r)
        live[k]["o"] = (o * r).astype(_BF)

    def stage_o(k):
        d = units[k]
        o = live[k].pop("o")
        step = _D // _OSPLIT
        parts = []
        for r in range(_OSPLIT):
            rows = slice(r * step, (r + 1) * step)
            res = _nt(d["wo"][rows, 0:_DH], o[0:_SQ]) + _nt(d["wo"][rows, _DH:_HP], o[_SQ:2 * _SQ])
            if not d["first"]:
                res = acc[d["u"], rows, :] + res
            if d["last"]:
                parts.append(res)
            else:
                acc[d["u"], rows, :] = res
        if d["last"]:
            live[k]["fin"] = jnp.concatenate(parts, axis=0)

    def put(b, j, t):
        r, s = tile_loc(b, j)
        pool[r, s:s + 128, :] = t.T.astype(_BF)
        pltpu.make_async_copy(pool.at[r, pl.ds(s, 128), :], out_hbm.at[b, :, pl.ds(j * 128, 128)], sem_o.at[0]).start()

    def stage_fa(b):
        for j in range(4):
            put(b, j, acc[b, j * 128:(j + 1) * 128, :])

    def stage_fb(k):
        b = units[k]["b"]
        fin = live[k].pop("fin")
        put(b, 4, jnp.concatenate([acc[b, 512:_D, :], fin[0:64]], axis=0))
        for j in range(4):
            put(b, 5 + j, fin[64 + j * 128:64 + (j + 1) * 128, :])

    stages = {"Q": stage_q, "TQ": stage_tq, "S": stage_s, "V": stage_v, "O": stage_o,
              "FA": stage_fa, "FB": stage_fb, "H": hook}

    def emit(seq):
        for name, a in seq:
            stages[name](a)

    def make_units(tag, br, kv, wo, q, first=False, last=False, qbase=None):
        keys = []
        for b in range(_B):
            u = br * _B + b
            units[(tag, b)] = dict(b=b, u=u, kv=kv, wo=wo, q=q, qi=u if qbase is None else qbase + b,
                                   first=first, last=last)
            keys.append((tag, b))
        return keys

    wq_a0, wq_b0, wo_a1 = w0.at[0], w0.at[1], w0.at[2]
    wq_a1, wq_b1, wo_a0, wo_b0 = wv.at[0, 0, 0], wv.at[0, 0, 1], wv.at[0, 1, 0], wv.at[0, 1, 1]
    nx0, nq1, cut = 4, 5, 5
    plan = [
        lambda s: [cp_w(0, 0, 0, wq_a0, s)] + [cp_x(0, b, b + 1, s) for b in range(nx0)],
        lambda s: [cp_x(0, nx0, _B, s), cp_w(1, 0, 0, wq_a1, s)],
        lambda s: [cp_w(0, 1, 0, wo_a0, s), cp_kv(0, 0, 0, 0, 0, cut, s), cp_kv(0, 0, 1, 0, 0, cut, s)],
        lambda s: [cp_kv(0, 0, 0, 0, cut, _B, s), cp_kv(0, 0, 1, 0, cut, _B, s), cp_w(0, 0, 1, wq_b0, s),
                   cp_x(1, 0, _B, s)],
        lambda s: [cp_w(0, 1, 1, wo_b0, s), cp_kv(0, 0, 0, 1, 0, _B, s), cp_kv(0, 0, 1, 1, 0, _B, s),
                   cp_w(1, 0, 1, wq_b1, s)],
        lambda s: [cp_kv(1, 0, 0, 0, 0, _B, s), cp_kv(1, 0, 1, 0, 0, _B, s), cp_w(1, 1, 0, wo_a1, s)],
    ]
    groups = [mk(sem_g.at[i % 3]) for i, mk in enumerate(plan)]
    nxt = block_copies(1, 1)
    groups += [nxt[:4], nxt[4:]]
    for i in range(6):
        hooks[i] = [functools.partial(wait_all, groups[i])]
        hooks.setdefault("a0" if i + 2 == 5 else i, []).append(functools.partial(start_all, groups[i + 2]))
    start_all(groups[0])
    start_all(groups[1])

    a0 = make_units("A0", 0, 0, wo_a0, q0, first=True, qbase=0)
    b0 = make_units("B0", 1, 0, wo_b0, qs, first=True)
    a1 = make_units("A1", 0, 0, wo_a1, qs)
    tq_a = [("TQ", (0, b, wq_a0, q0, b)) for b in range(_B)]
    tq_b = [("TQ", (1, b, wq_b0, qs, _B + b)) for b in range(_B)]
    q_a1 = [("Q", (0, b, wq_a1, qs, b)) for b in range(_B)]
    q_b1 = [("Q", (1, b, wq_b1, qs, _B + b)) for b in range(_B)]
    seq = [("H", 0)] + tq_a[:nx0] + [("H", 1)] + q_a1[:2] + tq_a[nx0:] + q_a1[2:nq1] + [("H", 2)]
    part, pend = _interleave(a0[:cut], q_a1[nq1:nq1 + 2], q_a1[nq1 + 2:], [])
    seq += part + [("H", 3)]
    part, pend = _interleave(a0[cut:], [], tq_b, pend)
    seq += part + [("H", "a0"), ("H", 4)]
    part, pend = _interleave(b0, [], [], pend)
    for e in part:
        seq.append(e)
        if e[0] == "V" and e[1][1] < 4:
            seq.append(q_b1[e[1][1]])
    seq.append(("H", 5))
    part, pend = _interleave(a1, [], q_b1[4:], pend)
    emit(seq + part + [("O", k) for k in pend])
    assert not hooks

    def body(j, slot):
        nx = block_copies(j + 1, 1 - slot)
        wait_block(slot)
        bu = make_units("B", 1, slot, wv.at[slot, 1, 1], qs)
        au = make_units("A", 0, slot, wv.at[slot, 1, 0], qs)
        hooks[("S", bu[1])] = [functools.partial(start_all, nx[:4])]
        hooks[("S", bu[2])] = [functools.partial(start_all, nx[4:])]
        q_a = [("Q", (0, b, wv.at[slot, 0, 0], qs, b)) for b in range(_B)]
        q_b = [("Q", (1, b, wv.at[slot, 0, 1], qs, _B + b)) for b in range(_B)]
        part, pend = _interleave(bu + au, q_a[1:3], q_a[3:] + q_b, [])
        emit(q_a[:1] + part + [("O", k) for k in pend])
        return 1 - slot

    last_slot = jax.lax.fori_loop(1, _HKV - 1, body, 1)

    wait_block((_HKV - 1) % 2)
    lu = make_units("L", 1, last_slot, wv.at[(_HKV - 1) % 2, 1, 1], qs, last=True)
    part = [("S", lu[0])]
    for i in range(_B):
        if i + 1 < _B:
            part.append(("S", lu[i + 1]))
        if 1 <= i < _B - 1:
            part.append(("O", lu[i - 1]))
        part.append(("V", lu[i]))
    part += [("O", lu[_B - 2]), ("O", lu[_B - 1])]
    seq, due, fa_left = [], [], list(range(_B))
    for n, e in enumerate(part):
        seq.append(e)
        if fa_left and n >= 1:
            seq.append(("FA", fa_left.pop(0)))
        due = [(c - 1, k) for c, k in due]
        while due and due[0][0] <= 0:
            seq.append(("FB", due.pop(0)[1]))
        if e[0] == "O":
            due.append((_FIN_LAG, e[1]))
    emit(seq + [("FB", k) for _, k in due])
    staged = pool.at[pl.ds(_KV_ROWS, _OUT_ROWS)]
    pltpu.make_async_copy(staged, staged, sem_o.at[0]).wait()


@jax.jit
def pallas_concat_heads__gqa_block_cached__gqa_block_cached__near_ridge_kernel(
    A_x: jax.Array,
    A_k_cache: jax.Array,
    A_v_cache: jax.Array,
    A_wq: jax.Array,
    A_wo: jax.Array,
    B_x: jax.Array,
    B_k_cache: jax.Array,
    B_v_cache: jax.Array,
    B_wq: jax.Array,
    B_wo: jax.Array,
):
    hbm = pl.BlockSpec(memory_space=pltpu.HBM)
    return pl.pallas_call(
        _kernel,
        in_specs=[hbm] * 10,
        out_specs=hbm,
        out_shape=jax.ShapeDtypeStruct((_B, _SQ, 2 * _D), _BF),
        scratch_shapes=[
            pltpu.VMEM((2 * _B, _D, _SQ), _BF),
            pltpu.VMEM((2 * _B, _SQ, _DP), _BF),
            pltpu.VMEM((2 * _B, 2 * _SQ, _DH), _BF),
            pltpu.VMEM((_B, 2 * _SQ, _DH), _BF),
            pltpu.VMEM((_KV_ROWS + _OUT_ROWS, _SK, _DH), _BF),
            pltpu.VMEM((2, 2, 2, _D, _HP), _BF),
            pltpu.VMEM((3, _D, _HP), _BF),
            pltpu.VMEM((2 * _B, _D, _SQ), jnp.float32),
            pltpu.SemaphoreType.DMA((3,)),
            pltpu.SemaphoreType.DMA((2,)),
            pltpu.SemaphoreType.DMA((2,)),
            pltpu.SemaphoreType.DMA((1,)),
        ],
        compiler_params=pltpu.CompilerParams(vmem_limit_bytes=100 * 1024 * 1024, disable_bounds_checks=True),
    )(
        A_x.transpose(0, 2, 1), A_k_cache, A_v_cache, A_wq, A_wo.T,
        B_x.transpose(0, 2, 1), B_k_cache, B_v_cache, B_wq, B_wo.T,
    )
```
